```python
import os as _os
_os.environ.setdefault("JAX_PLATFORMS", "cpu")
import jax
import jax.numpy as jnp

def _softmax(x, axis=-1):
    return jax.nn.softmax(x, axis=axis)
def _gelu(x):
    return jax.nn.gelu(x, approximate=True)
def _silu(x):
    return jax.nn.silu(x)
def _sigmoid(x):
    return jax.nn.sigmoid(x)
def _layernorm(x, axis=-1, eps=1e-5):
    m = jnp.mean(x, axis=axis, keepdims=True)
    v = jnp.var(x, axis=axis, keepdims=True)
    return (x - m) / jnp.sqrt(v + eps)
def _scatter_add(tgt, idx, src, axis=0):
    return tgt.at[idx].add(src)
def _segment_sum(src, seg, n):
    return jax.ops.segment_sum(src, seg, n)
class _Rng:
    def __init__(self, key):
        self._k = key
    def _next(self):
        self._k, sub = jax.random.split(self._k)
        return sub
    def normal(self, shape):
        return jax.random.normal(self._next(), shape, dtype=jnp.bfloat16)
    def randint(self, lo, hi, shape):
        return jax.random.randint(self._next(), shape, lo, hi, dtype=jnp.int32)
    def uniform(self, shape, lo=0.0, hi=1.0):
        return jax.random.uniform(self._next(), shape, jnp.bfloat16, lo, hi)
    def permutation(self, n):
        return jax.random.permutation(self._next(), n)


kernel_name = 'concat_heads__gqa_block_cached__gqa_block_cached__near_ridge'

def setup_inputs():
    _rng = _Rng(jax.random.key(int.from_bytes(__import__("os").urandom(4), "little")))
    _w = (lambda a: (lambda t: t.astype(jnp.bfloat16) if jnp.issubdtype(t.dtype, jnp.floating) else t)(jnp.asarray(a)))
    def _A_setup():
        B, Sq, D = 8, 128, 576
        Hq, Hkv, Sk, Dh = 32, 16, 512, 128
        assert Hq % Hkv == 0, (Hq, Hkv)
        return {
            "x": _w((lambda *s: _rng.normal(s) * 0.8)(B, Sq, D)),
            "k_cache": _w((lambda *s: _rng.normal(s) * 0.8)(B, Hkv, Sk, Dh)),
            "v_cache": _w((lambda *s: _rng.normal(s) * 0.05)(B, Hkv, Sk, Dh)),
            "wq": _w((lambda *s: _rng.normal(s) * 0.8)(D, Hq * Dh) * (D ** -0.5)),
            "wo": _w((lambda *s: _rng.normal(s) * 0.05)(Hq * Dh, D) * ((Hq * Dh) ** -0.5)),
        }
    _A_in = _A_setup()

    def _B_setup():
        B, Sq, D = 8, 128, 576
        Hq, Hkv, Sk, Dh = 32, 16, 512, 128
        assert Hq % Hkv == 0, (Hq, Hkv)
        return {
            "x": _w((lambda *s: _rng.normal(s) * 0.8)(B, Sq, D)),
            "k_cache": _w((lambda *s: _rng.normal(s) * 0.8)(B, Hkv, Sk, Dh)),
            "v_cache": _w((lambda *s: _rng.normal(s) * 0.05)(B, Hkv, Sk, Dh)),
            "wq": _w((lambda *s: _rng.normal(s) * 0.8)(D, Hq * Dh) * (D ** -0.5)),
            "wo": _w((lambda *s: _rng.normal(s) * 0.05)(Hq * Dh, D) * ((Hq * Dh) ** -0.5)),
        }
    _B_in = _B_setup()

    return {
        "A_x": _A_in["x"],
        "A_k_cache": _A_in["k_cache"],
        "A_v_cache": _A_in["v_cache"],
        "A_wq": _A_in["wq"],
        "A_wo": _A_in["wo"],
        "B_x": _B_in["x"],
        "B_k_cache": _B_in["k_cache"],
        "B_v_cache": _B_in["v_cache"],
        "B_wq": _B_in["wq"],
        "B_wo": _B_in["wo"],
    }

def reference(A_x, A_k_cache, A_v_cache, A_wq, A_wo, B_x, B_k_cache, B_v_cache, B_wq, B_wo):
    def _A_ref(x, k_cache, v_cache, wq, wo):
        B, Sq, D = x.shape
        Hq, Dh = 32, 128
        Hkv = k_cache.shape[1]
        rep = Hq // Hkv
        q = (lambda x, *d: x.transpose(*d))((x @ wq).reshape(B, Sq, Hq, Dh), 0, 2, 1, 3)
        k = jnp.repeat(k_cache, rep, axis=1)
        v = jnp.repeat(v_cache, rep, axis=1)
        scores = jnp.einsum("bhqd,bhkd->bhqk", q, k) * (Dh ** -0.5)
        p = _softmax(scores, axis=-1)
        o = jnp.einsum("bhqk,bhkd->bhqd", p, v)
        return (lambda x, *d: x.transpose(*d))(o, 0, 2, 1, 3).reshape(B, Sq, Hq * Dh) @ wo

    def _B_ref(x, k_cache, v_cache, wq, wo):
        B, Sq, D = x.shape
        Hq, Dh = 32, 128
        Hkv = k_cache.shape[1]
        rep = Hq // Hkv
        q = (lambda x, *d: x.transpose(*d))((x @ wq).reshape(B, Sq, Hq, Dh), 0, 2, 1, 3)
        k = jnp.repeat(k_cache, rep, axis=1)
        v = jnp.repeat(v_cache, rep, axis=1)
        scores = jnp.einsum("bhqd,bhkd->bhqk", q, k) * (Dh ** -0.5)
        p = _softmax(scores, axis=-1)
        o = jnp.einsum("bhqk,bhkd->bhqd", p, v)
        return (lambda x, *d: x.transpose(*d))(o, 0, 2, 1, 3).reshape(B, Sq, Hq * Dh) @ wo

    a = _A_ref(A_x, A_k_cache, A_v_cache, A_wq, A_wo)
    b = _B_ref(B_x, B_k_cache, B_v_cache, B_wq, B_wo)
    return jnp.concatenate([a, b], axis=-1)
```

```python
import functools

import jax
import jax.numpy as jnp
from jax import lax
import jax.experimental.pallas as pl
import jax.experimental.pallas.tpu as pltpu

B, SQ, D = 8, 128, 576
HQ, HKV, SK, DH = 32, 16, 512, 128
REP = HQ // HKV
M = B * SQ
NQ = HQ * DH
NS = 4
LOG2E = 1.4426950408889634
WQ_SPLITS = (0, 512, 1536, 4096)
OUT_CHUNKS = 4
OUT_CM = M // OUT_CHUNKS


def _kernel(xa, ka, va, wqa, woa, xb, kb, vb, wqb, wob, out_hbm,
            x_buf, wq_buf, wo_buf, k_buf, v_buf, q_scr, o_scr, xn_scr, out_buf,
            x_sem, wq_sem, wo_sem, k_sem, v_sem, out_sem):
    xs_hbm = (xa, xb)
    ks_hbm = (ka, kb)
    vs_hbm = (va, vb)
    wqs_hbm = (wqa, wqb)
    wos_hbm = (woa, wob)
    scale = DH ** -0.5 * LOG2E
    nwq = len(WQ_SPLITS) - 1

    def x_copy(br):
        return pltpu.make_async_copy(xs_hbm[br], x_buf.at[br], x_sem.at[br])

    def wq_copy(br, j):
        lo, hi = WQ_SPLITS[j], WQ_SPLITS[j + 1]
        return pltpu.make_async_copy(
            wqs_hbm[br].at[:, pl.ds(lo, hi - lo)],
            wq_buf.at[br, :, pl.ds(lo, hi - lo)],
            wq_sem.at[br, j])

    def wo_copy(br):
        return pltpu.make_async_copy(wos_hbm[br], wo_buf.at[br], wo_sem.at[br])

    def kv_copies(br, b, slot):
        return (pltpu.make_async_copy(ks_hbm[br].at[b], k_buf.at[slot], k_sem.at[slot]),
                pltpu.make_async_copy(vs_hbm[br].at[b], v_buf.at[slot], v_sem.at[slot]))

    def out_copy(i):
        return pltpu.make_async_copy(out_buf.at[pl.ds(i * OUT_CM, OUT_CM), :],
                                     out_hbm.at[pl.ds(i * OUT_CM, OUT_CM), :],
                                     out_sem.at[i])

    def transpose_x(br):
        for b in range(B):
            xn_scr[br, b * SQ:(b + 1) * SQ, :] = x_buf[br, b].T

    def qproj(br, lo, hi):
        res = jnp.dot(xn_scr[br], wq_buf[br, :, lo:hi], preferred_element_type=jnp.float32)
        res = (res * scale).astype(jnp.bfloat16)
        for b in range(B):
            for c in range((hi - lo) // DH):
                head = lo // DH + c
                q_scr[b * HKV + head // REP, (head % REP) * SQ:(head % REP + 1) * SQ, :] = (
                    res[b * SQ:(b + 1) * SQ, c * DH:(c + 1) * DH])

    x_copy(0).start()
    wq_copy(0, 0).start()

    for br in range(2):
        with jax.named_scope('phase1'):
            if br == 0:
                x_copy(0).wait()
                wq_copy(0, 1).start()
                transpose_x(0)
                wq_copy(0, 0).wait()
                wq_copy(0, 2).start()
                qproj(0, WQ_SPLITS[0], WQ_SPLITS[1])
                wq_copy(0, 1).wait()
                for s in range(2):
                    for c in kv_copies(0, s, s):
                        c.start()
                qproj(0, WQ_SPLITS[1], WQ_SPLITS[2])
                wq_copy(0, 2).wait()
                for s in range(2, NS):
                    for c in kv_copies(0, s, s):
                        c.start()
                wo_copy(0).start()
                qproj(0, WQ_SPLITS[2], WQ_SPLITS[3])
            else:
                for j in range(nwq):
                    wq_copy(1, j).wait()
                wo_copy(1).start()
                qproj(1, 0, NQ)

        with jax.named_scope('phase2'):
            def batch_body(b, carry, br=br):
                slot = lax.rem(b, NS)
                for c in kv_copies(br, b, slot):
                    c.wait()
                r0 = pl.multiple_of(b * SQ, SQ)
                for h in range(HKV):
                    q2 = q_scr[b * HKV + h]
                    k = k_buf[slot, h]
                    v = v_buf[slot, h]
                    s = lax.dot_general(q2, k, (((1,), (1,)), ((), ())),
                                        preferred_element_type=jnp.float32)
                    m = jnp.max(s, axis=-1, keepdims=True)
                    p = jnp.exp2(s - m)
                    l = jnp.sum(p, axis=-1, keepdims=True)
                    o = jnp.dot(p.astype(jnp.bfloat16), v, preferred_element_type=jnp.float32)
                    r = pl.reciprocal(l, approx=True)
                    r = r * (2.0 - l * r)
                    o = (o * r).astype(jnp.bfloat16)
                    c0 = h * REP * DH
                    o_scr[pl.ds(r0, SQ), c0:c0 + DH] = o[:SQ]
                    o_scr[pl.ds(r0, SQ), c0 + DH:c0 + 2 * DH] = o[SQ:]

                @pl.when(b < B - NS)
                def _():
                    for c in kv_copies(br, b + NS, slot):
                        c.start()

                if br == 0:
                    @pl.when(b >= B - NS)
                    def _():
                        for c in kv_copies(1, b - (B - NS), slot):
                            c.start()

                    @pl.when(b == 1)
                    def _():
                        x_copy(1).start()
                        for j in range(nwq):
                            wq_copy(1, j).start()
                return carry

            lax.fori_loop(0, B, batch_body, 0)

        with jax.named_scope('phase3'):
            wo_copy(br).wait()
            if br == 0:
                x_copy(1).wait()
                transpose_x(1)
                res = lax.dot_general(o_scr[...], wo_buf[br], (((1,), (1,)), ((), ())),
                                      preferred_element_type=jnp.float32)
                out_buf[:, 0:D] = res.astype(out_buf.dtype)
            else:
                for i in range(OUT_CHUNKS):
                    res = lax.dot_general(o_scr[i * OUT_CM:(i + 1) * OUT_CM, :], wo_buf[br],
                                          (((1,), (1,)), ((), ())),
                                          preferred_element_type=jnp.float32)
                    out_buf[i * OUT_CM:(i + 1) * OUT_CM, D:2 * D] = res.astype(out_buf.dtype)
                    out_copy(i).start()
                for i in range(OUT_CHUNKS):
                    out_copy(i).wait()


@jax.jit
def pallas_concat_heads__gqa_block_cached__gqa_block_cached__near_ridge_kernel(
    A_x, A_k_cache, A_v_cache, A_wq, A_wo,
    B_x, B_k_cache, B_v_cache, B_wq, B_wo,
):
    bf16 = jnp.bfloat16
    hbm_spec = pl.BlockSpec(memory_space=pltpu.HBM)
    out = pl.pallas_call(
        _kernel,
        out_shape=jax.ShapeDtypeStruct((M, 2 * D), bf16),
        in_specs=[hbm_spec] * 10,
        out_specs=hbm_spec,
        scratch_shapes=[
            pltpu.VMEM((2, B, D, SQ), bf16),
            pltpu.VMEM((2, D, NQ), bf16),
            pltpu.VMEM((2, D, NQ), bf16),
            pltpu.VMEM((NS, HKV, SK, DH), bf16),
            pltpu.VMEM((NS, HKV, SK, DH), bf16),
            pltpu.VMEM((B * HKV, REP * SQ, DH), bf16),
            pltpu.VMEM((M, NQ), bf16),
            pltpu.VMEM((2, M, D), bf16),
            pltpu.VMEM((M, 2 * D), bf16),
            pltpu.SemaphoreType.DMA((2,)),
            pltpu.SemaphoreType.DMA((2, len(WQ_SPLITS) - 1)),
            pltpu.SemaphoreType.DMA((2,)),
            pltpu.SemaphoreType.DMA((NS,)),
            pltpu.SemaphoreType.DMA((NS,)),
            pltpu.SemaphoreType.DMA((OUT_CHUNKS,)),
        ],
        compiler_params=pltpu.CompilerParams(vmem_limit_bytes=110 * 1024 * 1024),
    )(A_x.transpose(0, 2, 1), A_k_cache, A_v_cache, A_wq, A_wo.T,
      B_x.transpose(0, 2, 1), B_k_cache, B_v_cache, B_wq, B_wo.T)
    return out.reshape(B, SQ, 2 * D)
```

```python
import jax
import jax.numpy as jnp
from jax import lax
import jax.experimental.pallas as pl
import jax.experimental.pallas.tpu as pltpu

B, SQ, D = 8, 128, 576
HQ, HKV, SK, DH = 32, 16, 512, 128
REP = HQ // HKV
M = B * SQ
NQ = HQ * DH
LOG2E = 1.4426950408889634
WQ_SPLITS = (0, 512, 1536, 4096)
OUT_SPLITS = (0, 512, 896, 1024)
OUT_CHUNKS = len(OUT_SPLITS) - 1
DA = (D // 128) * 128


def _kernel(xa, ka, va, wqa, woa, xb, kb, vb, wqb, wob, out_hbm,
            x_buf, wq_buf, wo_buf, k_buf, v_buf, q_scr, o_scr, xn_scr, out_buf, tail_scr,
            fence_buf,
            x_sem, wq_sem, wo_sem, k_sem, v_sem, out_sem, fence_sem):
    xs_hbm = (xa, xb)
    ks_hbm = (ka, kb)
    vs_hbm = (va, vb)
    wqs_hbm = (wqa, wqb)
    wos_hbm = (woa, wob)
    scale = DH ** -0.5 * LOG2E
    nwq = len(WQ_SPLITS) - 1

    def x_copy(br):
        return pltpu.make_async_copy(xs_hbm[br], x_buf.at[br], x_sem.at[br])

    def wq_copy(br, j):
        lo, hi = WQ_SPLITS[j], WQ_SPLITS[j + 1]
        return pltpu.make_async_copy(
            wqs_hbm[br].at[:, pl.ds(lo, hi - lo)],
            wq_buf.at[br, :, pl.ds(lo, hi - lo)],
            wq_sem.at[br, j])

    def wo_copy(br):
        return pltpu.make_async_copy(wos_hbm[br], wo_buf.at[br], wo_sem.at[br])

    def kv_copies(br, b):
        return (pltpu.make_async_copy(ks_hbm[br].at[b], k_buf.at[b], k_sem.at[b]),
                pltpu.make_async_copy(vs_hbm[br].at[b], v_buf.at[b], v_sem.at[b]))

    def start_kv(br, bs):
        for b in bs:
            for c in kv_copies(br, b):
                c.start()

    def wait_kv(br, bs):
        for b in bs:
            for c in kv_copies(br, b):
                c.wait()

    def out_copy(i):
        lo, hi = OUT_SPLITS[i], OUT_SPLITS[i + 1]
        return pltpu.make_async_copy(out_buf.at[pl.ds(lo, hi - lo), :],
                                     out_hbm.at[pl.ds(lo, hi - lo), :],
                                     out_sem.at[i])

    def fence_copy(i):
        return pltpu.make_async_copy(xb.at[0, pl.ds(0, 16), :], fence_buf.at[i], fence_sem.at[i])

    def transpose_x(br):
        for b in range(B):
            xn_scr[br, b * SQ:(b + 1) * SQ, :] = x_buf[br, b].T

    def qproj(br, lo, hi):
        res = jnp.dot(xn_scr[br], wq_buf[br, :, lo:hi], preferred_element_type=jnp.float32)
        res = (res * scale).astype(jnp.bfloat16)
        for b in range(B):
            for c in range((hi - lo) // DH):
                head = lo // DH + c
                q_scr[b * HKV + head // REP, (head % REP) * SQ:(head % REP + 1) * SQ, :] = (
                    res[b * SQ:(b + 1) * SQ, c * DH:(c + 1) * DH])

    def scores(b, h):
        return lax.dot_general(q_scr[b * HKV + h], k_buf[b, h],
                               (((1,), (1,)), ((), ())),
                               preferred_element_type=jnp.float32)

    x_copy(0).start()
    wq_copy(0, 0).start()

    for br in range(2):
        if br == 0:
            x_copy(0).wait()
            wq_copy(0, 1).start()
            transpose_x(0)
            wq_copy(0, 0).wait()
            wq_copy(0, 2).start()
            qproj(0, WQ_SPLITS[0], WQ_SPLITS[1])
            wq_copy(0, 1).wait()
            start_kv(0, (0, 1))
            qproj(0, WQ_SPLITS[1], WQ_SPLITS[2])
            wq_copy(0, 2).wait()
            start_kv(0, (2, 3))
            qproj(0, WQ_SPLITS[2], WQ_SPLITS[3])
        else:
            qproj(1, 0, NQ)

        def pair_body(i, carry, br=br):
            b0 = 2 * i
            if br == 0:
                wait_kv(0, (b0, b0 + 1))

                @pl.when(i == 0)
                def _():
                    start_kv(0, (4, 5, 6, 7))

                @pl.when(i == 2)
                def _():
                    wo_copy(0).start()
                    x_copy(1).start()
                    for j in range(nwq):
                        wq_copy(1, j).start()

                @pl.when(i == 3)
                def _():
                    start_kv(1, (0, 1, 2, 3))
            else:
                @pl.when(i == 2)
                def _():
                    wait_kv(1, (4, 5, 6, 7))
                    wo_copy(1).wait()
            s_next = scores(b0, 0)
            for bb in range(2):
                b = b0 + bb
                rows = pl.ds(pl.multiple_of(b * SQ, SQ), SQ)
                for h in range(HKV):
                    s = s_next
                    if h + 1 < HKV:
                        s_next = scores(b, h + 1)
                    elif bb == 0:
                        s_next = scores(b + 1, 0)
                    v = v_buf[b, h]
                    m = jnp.max(s, axis=-1, keepdims=True)
                    p = jnp.exp2(s - m)
                    l = jnp.sum(p, axis=-1, keepdims=True)
                    o = jnp.dot(p.astype(jnp.bfloat16), v, preferred_element_type=jnp.float32)
                    r = pl.reciprocal(l, approx=True)
                    r = r * (2.0 - l * r)
                    o = (o * r).astype(jnp.bfloat16)
                    c0 = h * REP * DH
                    o_scr[rows, c0:c0 + DH] = o[:SQ]
                    o_scr[rows, c0 + DH:c0 + 2 * DH] = o[SQ:]
            return carry

        lax.fori_loop(0, B // 2, pair_body, 0)

        if br == 0:
            wo_copy(0).wait()
            x_copy(1).wait()
            for j in range(nwq):
                wq_copy(1, j).wait()
            start_kv(1, (4, 5, 6, 7))
            wo_copy(1).start()
            transpose_x(1)
        else:
            for i in range(OUT_CHUNKS - 1):
                fence_copy(i).start()
        for i in range(OUT_CHUNKS):
            rows = slice(OUT_SPLITS[i], OUT_SPLITS[i + 1])
            res_t = lax.dot_general(wo_buf[br], o_scr[rows, :], (((1,), (1,)), ((), ())),
                                    preferred_element_type=jnp.float32).astype(jnp.bfloat16)
            if br == 0:
                out_buf[rows, 0:DA] = res_t[:DA].T
                tail_scr[:, rows] = res_t[DA:]
            else:
                comb = jnp.concatenate([tail_scr[:, rows], res_t], axis=0)
                out_buf[rows, DA:2 * D] = comb.T
                out_copy(i).start()
                if i < OUT_CHUNKS - 1:
                    fence_copy(i).wait()
        if br == 0:
            wait_kv(1, (0, 1, 2, 3))
        else:
            for i in range(OUT_CHUNKS):
                out_copy(i).wait()


@jax.jit
def pallas_concat_heads__gqa_block_cached__gqa_block_cached__near_ridge_kernel(
    A_x, A_k_cache, A_v_cache, A_wq, A_wo,
    B_x, B_k_cache, B_v_cache, B_wq, B_wo,
):
    bf16 = jnp.bfloat16
    hbm_spec = pl.BlockSpec(memory_space=pltpu.HBM)
    out = pl.pallas_call(
        _kernel,
        out_shape=jax.ShapeDtypeStruct((M, 2 * D), bf16),
        in_specs=[hbm_spec] * 10,
        out_specs=hbm_spec,
        scratch_shapes=[
            pltpu.VMEM((2, B, D, SQ), bf16),
            pltpu.VMEM((2, D, NQ), bf16),
            pltpu.VMEM((2, D, NQ), bf16),
            pltpu.VMEM((B, HKV, SK, DH), bf16),
            pltpu.VMEM((B, HKV, SK, DH), bf16),
            pltpu.VMEM((B * HKV, REP * SQ, DH), bf16),
            pltpu.VMEM((M, NQ), bf16),
            pltpu.VMEM((2, M, D), bf16),
            pltpu.VMEM((M, 2 * D), bf16),
            pltpu.VMEM((D - DA, M), bf16),
            pltpu.VMEM((OUT_CHUNKS - 1, 16, SQ), bf16),
            pltpu.SemaphoreType.DMA((2,)),
            pltpu.SemaphoreType.DMA((2, len(WQ_SPLITS) - 1)),
            pltpu.SemaphoreType.DMA((2,)),
            pltpu.SemaphoreType.DMA((B,)),
            pltpu.SemaphoreType.DMA((B,)),
            pltpu.SemaphoreType.DMA((OUT_CHUNKS,)),
            pltpu.SemaphoreType.DMA((OUT_CHUNKS - 1,)),
        ],
        compiler_params=pltpu.CompilerParams(vmem_limit_bytes=120 * 1024 * 1024),
    )(A_x.transpose(0, 2, 1), A_k_cache, A_v_cache, A_wq, A_wo.T,
      B_x.transpose(0, 2, 1), B_k_cache, B_v_cache, B_wq, B_wo.T)
    return out.reshape(B, SQ, 2 * D)
```

```python
import jax
import jax.numpy as jnp
from jax import lax
import jax.experimental.pallas as pl
import jax.experimental.pallas.tpu as pltpu

B, SQ, D = 8, 128, 576
HQ, HKV, SK, DH = 32, 16, 512, 128
REP = HQ // HKV
M = B * SQ
NQ = HQ * DH
LOG2E = 1.4426950408889634
WQ_SPLITS = (0, 512, 1536, 4096)
OUT_SPLITS = (0, 512, 896, 1024)
OUT_CHUNKS = len(OUT_SPLITS) - 1
KV_GROUP = (2, 4)
DA = (D // 128) * 128


def _kernel(xa, ka, va, wqa, woa, xb, kb, vb, wqb, wob, out_hbm,
            x_buf, wq_buf, wo_buf, k_buf, v_buf, q_scr, o_scr, xn_scr, out_buf, tail_scr,
            fence_buf,
            x_sem, wq_sem, wo_sem, k_sem, v_sem, out_sem, fence_sem):
    xs_hbm = (xa, xb)
    ks_hbm = (ka, kb)
    vs_hbm = (va, vb)
    wqs_hbm = (wqa, wqb)
    wos_hbm = (woa, wob)
    scale = DH ** -0.5 * LOG2E
    nwq = len(WQ_SPLITS) - 1

    def x_copy(br):
        return pltpu.make_async_copy(xs_hbm[br], x_buf.at[br], x_sem.at[br])

    def wq_copy(br, j):
        lo, hi = WQ_SPLITS[j], WQ_SPLITS[j + 1]
        return pltpu.make_async_copy(
            wqs_hbm[br].at[:, pl.ds(lo, hi - lo)],
            wq_buf.at[br, :, pl.ds(lo, hi - lo)],
            wq_sem.at[br, j])

    def wo_copy(br):
        return pltpu.make_async_copy(wos_hbm[br], wo_buf.at[br], wo_sem.at[br])

    def kv_copies(br, g):
        n = KV_GROUP[br]
        sl = pl.ds(g * n, n)
        return (pltpu.make_async_copy(ks_hbm[br].at[sl], k_buf.at[sl], k_sem.at[br, g]),
                pltpu.make_async_copy(vs_hbm[br].at[sl], v_buf.at[sl], v_sem.at[br, g]))

    def start_kv(br, gs):
        for g in gs:
            for c in kv_copies(br, g):
                c.start()

    def wait_kv(br, gs):
        for g in gs:
            for c in kv_copies(br, g):
                c.wait()

    def wqb_copy():
        return pltpu.make_async_copy(wqb, wq_buf.at[1], wq_sem.at[1, 0])

    def out_copy(i):
        lo, hi = OUT_SPLITS[i], OUT_SPLITS[i + 1]
        return pltpu.make_async_copy(out_buf.at[pl.ds(lo, hi - lo), :],
                                     out_hbm.at[pl.ds(lo, hi - lo), :],
                                     out_sem.at[i])

    def fence_copy(i):
        return pltpu.make_async_copy(xb.at[0, pl.ds(0, 16), :], fence_buf.at[i], fence_sem.at[i])

    def transpose_x(br):
        for b in range(B):
            xn_scr[br, b * SQ:(b + 1) * SQ, :] = x_buf[br, b].T

    def qproj(br, lo, hi):
        res = jnp.dot(xn_scr[br], wq_buf[br, :, lo:hi], preferred_element_type=jnp.float32)
        res = (res * scale).astype(jnp.bfloat16)
        for b in range(B):
            for c in range((hi - lo) // DH):
                head = lo // DH + c
                q_scr[b * HKV + head // REP, (head % REP) * SQ:(head % REP + 1) * SQ, :] = (
                    res[b * SQ:(b + 1) * SQ, c * DH:(c + 1) * DH])

    def scores(b, h):
        return lax.dot_general(q_scr[b * HKV + h], k_buf[b, h],
                               (((1,), (1,)), ((), ())),
                               preferred_element_type=jnp.float32)

    x_copy(0).start()
    wq_copy(0, 0).start()

    for br in range(2):
        if br == 0:
            x_copy(0).wait()
            wq_copy(0, 1).start()
            transpose_x(0)
            wq_copy(0, 0).wait()
            wq_copy(0, 2).start()
            qproj(0, WQ_SPLITS[0], WQ_SPLITS[1])
            wq_copy(0, 1).wait()
            start_kv(0, (0,))
            qproj(0, WQ_SPLITS[1], WQ_SPLITS[2])
            wq_copy(0, 2).wait()
            start_kv(0, (1,))
            qproj(0, WQ_SPLITS[2], WQ_SPLITS[3])
        else:
            qproj(1, 0, NQ)

        nb = 2 if br == 0 else 4

        def pair_body(i, carry, br=br, nb=nb):
            b0 = nb * i
            if br == 0:
                wait_kv(0, (i,))

                @pl.when(i == 0)
                def _():
                    start_kv(0, (2, 3))

                @pl.when(i == 2)
                def _():
                    wo_copy(0).start()
                    x_copy(1).start()
                    wqb_copy().start()

                @pl.when(i == 3)
                def _():
                    start_kv(1, (0,))
            else:
                @pl.when(i == 1)
                def _():
                    wait_kv(1, (1,))
                    wo_copy(1).wait()
            s_next = scores(b0, 0)
            for bb in range(nb):
                b = b0 + bb
                rows = pl.ds(pl.multiple_of(b * SQ, SQ), SQ)
                for h in range(HKV):
                    s = s_next
                    if h + 1 < HKV:
                        s_next = scores(b, h + 1)
                    elif bb + 1 < nb:
                        s_next = scores(b + 1, 0)
                    v = v_buf[b, h]
                    m = jnp.max(s, axis=-1, keepdims=True)
                    p = jnp.exp2(s - m)
                    l = jnp.sum(p, axis=-1, keepdims=True)
                    o = jnp.dot(p.astype(jnp.bfloat16), v, preferred_element_type=jnp.float32)
                    r = pl.reciprocal(l, approx=True)
                    r = r * (2.0 - l * r)
                    o = (o * r).astype(jnp.bfloat16)
                    c0 = h * REP * DH
                    o_scr[rows, c0:c0 + DH] = o[:SQ]
                    o_scr[rows, c0 + DH:c0 + 2 * DH] = o[SQ:]
            return carry

        lax.fori_loop(0, B // nb, pair_body, 0)

        if br == 0:
            wo_copy(0).wait()
            x_copy(1).wait()
            wqb_copy().wait()
            start_kv(1, (1,))
            wo_copy(1).start()
            transpose_x(1)
        else:
            for i in range(OUT_CHUNKS - 1):
                fence_copy(i).start()
        for i in range(OUT_CHUNKS):
            rows = slice(OUT_SPLITS[i], OUT_SPLITS[i + 1])
            res_t = lax.dot_general(wo_buf[br], o_scr[rows, :], (((1,), (1,)), ((), ())),
                                    preferred_element_type=jnp.float32).astype(jnp.bfloat16)
            if br == 0:
                out_buf[rows, 0:DA] = res_t[:DA].T
                tail_scr[:, rows] = res_t[DA:]
            else:
                comb = jnp.concatenate([tail_scr[:, rows], res_t], axis=0)
                out_buf[rows, DA:2 * D] = comb.T
                out_copy(i).start()
                if i < OUT_CHUNKS - 1:
                    fence_copy(i).wait()
        if br == 0:
            wait_kv(1, (0,))
        else:
            for i in range(OUT_CHUNKS):
                out_copy(i).wait()


@jax.jit
def pallas_concat_heads__gqa_block_cached__gqa_block_cached__near_ridge_kernel(
    A_x, A_k_cache, A_v_cache, A_wq, A_wo,
    B_x, B_k_cache, B_v_cache, B_wq, B_wo,
):
    bf16 = jnp.bfloat16
    hbm_spec = pl.BlockSpec(memory_space=pltpu.HBM)
    out = pl.pallas_call(
        _kernel,
        out_shape=jax.ShapeDtypeStruct((M, 2 * D), bf16),
        in_specs=[hbm_spec] * 10,
        out_specs=hbm_spec,
        scratch_shapes=[
            pltpu.VMEM((2, B, D, SQ), bf16),
            pltpu.VMEM((2, D, NQ), bf16),
            pltpu.VMEM((2, D, NQ), bf16),
            pltpu.VMEM((B, HKV, SK, DH), bf16),
            pltpu.VMEM((B, HKV, SK, DH), bf16),
            pltpu.VMEM((B * HKV, REP * SQ, DH), bf16),
            pltpu.VMEM((M, NQ), bf16),
            pltpu.VMEM((2, M, D), bf16),
            pltpu.VMEM((M, 2 * D), bf16),
            pltpu.VMEM((D - DA, M), bf16),
            pltpu.VMEM((OUT_CHUNKS - 1, 16, SQ), bf16),
            pltpu.SemaphoreType.DMA((2,)),
            pltpu.SemaphoreType.DMA((2, len(WQ_SPLITS) - 1)),
            pltpu.SemaphoreType.DMA((2,)),
            pltpu.SemaphoreType.DMA((2, B // 2)),
            pltpu.SemaphoreType.DMA((2, B // 2)),
            pltpu.SemaphoreType.DMA((OUT_CHUNKS,)),
            pltpu.SemaphoreType.DMA((OUT_CHUNKS - 1,)),
        ],
        compiler_params=pltpu.CompilerParams(vmem_limit_bytes=120 * 1024 * 1024),
    )(A_x.transpose(0, 2, 1), A_k_cache, A_v_cache, A_wq, A_wo.T,
      B_x.transpose(0, 2, 1), B_k_cache, B_v_cache, B_wq, B_wo.T)
    return out.reshape(B, SQ, 2 * D)
```
